```python
import jax
import jax.numpy as jnp

def _softmax(x, axis=-1):
    return jax.nn.softmax(x, axis=axis)

def _gelu(x):
    return jax.nn.gelu(x, approximate=True)

def _silu(x):
    return jax.nn.silu(x)

def _sigmoid(x):
    return jax.nn.sigmoid(x)

def _layernorm(x, axis=-1, eps=1e-05):
    m = jnp.mean(x, axis=axis, keepdims=True)
    v = jnp.var(x, axis=axis, keepdims=True)
    return (x - m) / jnp.sqrt(v + eps)

def _scatter_add(tgt, idx, src, axis=0):
    return tgt.at[idx].add(src)

def _segment_sum(src, seg, n):
    return jax.ops.segment_sum(src, seg, n)

class _Rng:

    def __init__(self, key):
        self._k = key

    def _next(self):
        self._k, sub = jax.random.split(self._k)
        return sub

    def normal(self, shape):
        return jax.random.normal(self._next(), shape, dtype=jnp.bfloat16)

    def randint(self, lo, hi, shape):
        return jax.random.randint(self._next(), shape, lo, hi, dtype=jnp.int32)

    def uniform(self, shape, lo=0.0, hi=1.0):
        return jax.random.uniform(self._next(), shape, jnp.bfloat16, lo, hi)

    def permutation(self, n):
        return jax.random.permutation(self._next(), n)
kernel_name = 'adaLN_cond__spectral_gfnet__geglu_ffn__prompt'

def _fwd_setup_inputs():
    _rng = _Rng(jax.random.key(int.from_bytes(__import__("os").urandom(4), "little")))
    _w = lambda a: (lambda t: t.astype(jnp.bfloat16) if jnp.issubdtype(t.dtype, jnp.floating) else t)(jnp.asarray(a))

    def _A_setup():
        B, S, D = (1, 2048, 512)
        Df = D // 2 + 1
        return {'x': _w((lambda *s: _rng.normal(s) * 0.05)(B, S, D)), 'w_r': _w((lambda *s: _rng.normal(s) * 0.05)(S, Df) * 0.02), 'w_i': _w((lambda *s: _rng.normal(s) * 0.05)(S, Df) * 0.02)}
    _A_in = _A_setup()

    def _B_setup():
        B, S, D, F = (1, 2048, 512, 1792)
        return {'x': _w((lambda *s: _rng.normal(s) * 0.05)(B, S, D)), 'w_gate': _w((lambda *s: _rng.normal(s) * 0.05)(D, F)), 'w_up': _w((lambda *s: _rng.normal(s) * 0.05)(D, F)), 'w_down': _w((lambda *s: _rng.normal(s) * 0.05)(F, D))}
    _B_in = _B_setup()
    return {'A_x': _A_in['x'], 'A_w_r': _A_in['w_r'], 'A_w_i': _A_in['w_i'], 'B_x': _B_in['x'], 'B_w_gate': _B_in['w_gate'], 'B_w_up': _B_in['w_up'], 'B_w_down': _B_in['w_down'], 'c': _w((lambda *s: _rng.normal(s) * 0.05)(1, 512)), 'w_mod': _w((lambda *s: _rng.normal(s) * 0.05)(512, 6 * 512) * 512 ** (-0.5))}

def _fwd_reference(A_x, A_w_r, A_w_i, B_x, B_w_gate, B_w_up, B_w_down, c, w_mod):

    def _A_ref(x, w_r, w_i):
        B, S, D = x.shape
        X = (lambda x, axes=(-2, -1): jnp.fft.rfft2(x.astype(jnp.float32), axes=axes))(x, axes=(-2, -1))
        W = w_r + 1j * w_i
        X = X * W
        y = (lambda x, s, axes=(-2, -1): jnp.fft.irfft2(x, s=s, axes=axes).astype(jnp.bfloat16))(X, (S, D), axes=(-2, -1))
        return y

    def _B_ref(x, w_gate, w_up, w_down):
        return _gelu(x @ w_gate) * (x @ w_up) @ w_down
    x = A_x
    mod = (_silu(c) @ w_mod).reshape(c.shape[0], 6, 1, -1)
    sa, ca, ga, sb, cb, gb = (mod[:, 0].copy(), mod[:, 1].copy(), mod[:, 2].copy(), mod[:, 3].copy(), mod[:, 4].copy(), mod[:, 5].copy())
    h = _layernorm(x, axis=-1) * (1 + ca) + sa
    x = x + ga * _A_ref(h, A_w_r, A_w_i)
    h = _layernorm(x, axis=-1) * (1 + cb) + sb
    x = x + gb * _B_ref(h, B_w_gate, B_w_up, B_w_down)
    return x

def setup_inputs():
    _inp = _fwd_setup_inputs()
    _gk = jax.random.fold_in(jax.random.key(int.from_bytes(__import__("os").urandom(4), "little")), 2 ** 31 - 1)
    _shapes = [[1, 2048, 512]]
    _dtypes = ['bfloat16']
    _gks = jax.random.split(_gk, len(_shapes))
    _gs = [jax.random.normal(k, s, dtype=jnp.dtype(d)) * 0.05 for k, s, d in zip(_gks, _shapes, _dtypes)]
    _inp['grad_out'] = _gs[0]
    return _inp

def reference(A_x, A_w_r, A_w_i, B_w_gate, B_w_up, B_w_down, c, w_mod, B_x, grad_out):
    _const = dict(B_x=B_x)

    def _f(*_d):
        return _fwd_reference(**{'A_x': _d[0], 'A_w_r': _d[1], 'A_w_i': _d[2], 'B_w_gate': _d[3], 'B_w_up': _d[4], 'B_w_down': _d[5], 'c': _d[6], 'w_mod': _d[7], **_const})
    _out, _vjp = jax.vjp(_f, A_x, A_w_r, A_w_i, B_w_gate, B_w_up, B_w_down, c, w_mod)
    _grads = _vjp(grad_out)
    _out0 = jnp.asarray(_out)
    return (_out0, *[jnp.asarray(_g) for _g in _grads])
```

```python
import numpy as np
import jax
import jax.numpy as jnp
import jax.experimental.pallas as pl
import jax.experimental.pallas.tpu as pltpu

S, D, F = 2048, 512, 1792
DF = D // 2 + 1
R, N2 = 16, 128
P = S // 2
TOKEN = 15
MB = 64
SCALE = 2.0 / (S * D)
DH, FH = D // 2, F // 2
EPS = 1e-5
F32, BF16, U32 = jnp.float32, jnp.bfloat16, jnp.uint32
TP = 256

_G0 = float(np.sqrt(2.0 / np.pi))
_G1 = _G0 * 0.044715


def _constants():
    def dft(m, n):
        ang = 2 * np.pi * ((m[:, None] * np.arange(n)[None, :]) % D) / D
        return np.concatenate([np.cos(ang), -np.sin(ang)], axis=0)
    i = np.arange(64)
    cee, ceo = dft(4 * i, 128), dft(4 * i + 2, 128)
    cee[64] = 1.0 - 2.0 * (np.arange(128) % 2)
    j = np.arange(128)
    co = dft(MB * (j // (MB // 2)) + 4 * (j % (MB // 4)) + 1 + 2 * ((j // (MB // 4)) % 2), 256)
    weight = np.ones((128, 1))
    weight[0] = weight[64] = 0.5
    ce = np.stack([cee, ceo, weight * cee])
    k2 = np.arange(N2)[None, :]
    ang = 2 * np.pi * np.concatenate([(np.arange(N2)[:, None] * k2 % N2) / N2, np.arange(8 * R)[:, None] // 8 * k2 / S])
    ft = np.concatenate([np.cos(ang), -np.sin(ang)], axis=1).astype(np.float32)
    return ce.astype(jnp.bfloat16), co.astype(jnp.bfloat16), ft


_CE, _CO, _FT = _constants()


def _dft4(x, inv):
    (ar, ai), (br, bi), (cr, ci), (dr, di) = x
    s0r, s0i, d0r, d0i = ar + cr, ai + ci, ar - cr, ai - ci
    s1r, s1i, d1r, d1i = br + dr, bi + di, br - dr, bi - di
    p = (d0r + d1i, d0i - d1r)
    q = (d0r - d1i, d0i + d1r)
    return [(s0r + s1r, s0i + s1i), q if inv else p, (s0r - s1r, s0i - s1i), p if inv else q]


def _twiddle16(v, e, inv):
    r, i = v
    if e == 0:
        return v
    h = float(np.sqrt(0.5))
    if e == 4:
        return (-i, r) if inv else (i, -r)
    if e == 2:
        return ((r - i) * h, (r + i) * h) if inv else ((r + i) * h, (i - r) * h)
    if e == 6:
        return ((r + i) * (-h), (r - i) * h) if inv else ((i - r) * h, (r + i) * (-h))
    c = float(np.cos(2 * np.pi * e / 16))
    s = float(np.sin(2 * np.pi * e / 16)) * (1.0 if inv else -1.0)
    return (r * c - i * s, r * s + i * c)


def _dft16(x, inv):
    t = [_dft4([x[4 * a + b] for a in range(4)], inv) for b in range(4)]
    out = [None] * 16
    for c in range(4):
        col = _dft4([_twiddle16(t[b][c], b * c, inv) for b in range(4)], inv)
        for d in range(4):
            out[c + 4 * d] = col[d]
    return out


def _dot(a, b):
    return jnp.dot(a, b, preferred_element_type=F32)


def _mean(v):
    return jnp.sum(v, axis=-1, keepdims=True) * (1.0 / D)


def _colsum8(v):
    return jnp.sum(v.reshape(v.shape[0] // 8, 8, v.shape[1]), axis=0)


def _wide(v):
    return jnp.concatenate([v] * (D // 128), axis=1)


def _layernorm_bwd(dxhat, xhat, rstd):
    return rstd * (dxhat - _mean(dxhat) - xhat * _mean(dxhat * xhat))


def _ds(start, size):
    return pl.ds(start if isinstance(start, int) else pl.multiple_of(start, size), size)


class _Packed:
    def __init__(self, ref):
        self.ref = ref

    @staticmethod
    def _index(idx, packing):
        lead, rows, cols = (idx + (slice(None),))[:3] if isinstance(idx, tuple) else (idx, slice(None), slice(None))
        if isinstance(rows, tuple):
            rows = _ds(rows[0] * (rows[1] // packing), rows[1] // packing)
        elif rows != slice(None):
            rows = slice(rows.start // packing, rows.stop // packing)
        return lead, rows, cols

    def __getitem__(self, idx):
        return pltpu.bitcast(self.ref[self._index(idx, 2)], BF16)

    def __setitem__(self, idx, value):
        lead, rows, cols = self._index(idx, 1)
        self.ref.at[lead].bitcast(BF16)[rows, cols] = value.astype(BF16)


def _loop(name, lo, hi, streams):
    def body(i, carry):
        _weave(*streams(i))
        return carry
    with jax.named_scope(name):
        jax.lax.fori_loop(lo, hi, body, 0)


def _once(name, *streams):
    with jax.named_scope(name):
        _weave(*streams)


def _weave(*streams):
    steps = sorted(((k + 0.5) / n, s) for s, (_, n) in enumerate(streams) for k in range(n))
    for _, s in steps:
        next(streams[s][0])
    for gen, _ in streams:
        assert next(gen, 1) == 1


def _dot_nt(a, b):
    return jax.lax.dot_general(a, b, (((1,), (1,)), ((), ())), preferred_element_type=F32)


def _dot_tn(a, b):
    return jax.lax.dot_general(a, b, (((0,), (0,)), ((), ())), preferred_element_type=F32)


def _unpack(u):
    return pltpu.bitcast(u << 16, F32), pltpu.bitcast(u & jnp.uint32(0xFFFF0000), F32)


def _pack(lo, hi):
    lo = pltpu.bitcast(lo.astype(BF16).astype(F32), U32) >> 16
    return lo | pltpu.bitcast(hi.astype(BF16).astype(F32), U32)


def _lhs(a11, a12, a21, a22):
    return [a11 + a22, a21 + a22, a11, a22, a11 + a12, a21 - a11, a12 - a22]


def _rhs(b11, b12, b21, b22):
    return [b11 + b22, b11, b12 - b22, b21 - b11, b22, b11 + b12, b21 + b22]


def _out(m):
    return m[0] + m[3] - m[4] + m[6], m[2] + m[4], m[1] + m[3], m[0] - m[1] + m[2] + m[5]


def _out_t(c11, c12, c21, c22):
    return [c11 + c22, c21 - c22, c12 + c22, c11 + c21, c12 - c11, c22, c11]


def _lhs_t(m):
    return m[0] + m[2] + m[4] - m[5], m[4] + m[6], m[1] + m[5], m[0] + m[1] + m[3] - m[6]


def _rhs_t(m):
    return m[0] + m[1] - m[3] + m[5], m[2] + m[5], m[3] + m[6], m[0] - m[2] + m[4] + m[6]


def _kernel(x_hbm, wr_hbm, wi_hbm, wg_hbm, wu_hbm, wd_hbm, c_ref, wm_hbm, g_hbm,
            ce_ref, co_ref, ft_ref, zero_ref,
            out_hbm, dx_hbm, dwr_hbm, dwi_hbm, dwg_hbm, dwu_hbm, dwd_hbm, dc_ref, dwm_hbm,
            x32, g32, w32, wn_v, wg_v, wu_v, wd_v, wm_v, ms_v,
            xp_v, gp_v, y_v, u_v, xs_v, y1_v, x2_v,
            wgu_s, wd_s, h_s, ht_s, dy_s, dyt_s, da_v, a_s, dgu_s,
            mod_v, acc_v, dwn_v, stat_v, t_v, sem):
    (ms_v, y_v, u_v, wgu_s, wd_s, h_s, ht_s, dy_s, dyt_s, da_v, a_s, dgu_s) = map(_Packed, (
        ms_v, y_v, u_v, wgu_s, wd_s, h_s, ht_s, dy_s, dyt_s, da_v, a_s, dgu_s))
    groups = []

    def copy(*pairs):
        group = [pltpu.make_async_copy(src, dst, sem.at[len(groups)]) for src, dst in pairs]
        groups.append(group)
        return group

    def start(*new):
        for group in new:
            for cp in group:
                cp.start()

    def wait(*started):
        for group in started:
            for cp in group:
                cp.wait()

    tile = lambda q: slice(128 * q, 128 * q + 128)
    col = lambda j, n=1: slice(D * j, D * (j + n))
    ld_wm = lambda j, n: copy((wm_hbm.at[:, col(j, n)], wm_v.at[:, col(j, n)]))
    ld_wm0, ld_wm2, ld_wm5 = ld_wm(0, 2), ld_wm(2, 3), ld_wm(5, 1)
    ld_x = copy(*[(x_hbm.at[:, tile(q)], x32.at[q].bitcast(BF16)) for q in range(4)])
    ld_g = copy(*[(g_hbm.at[:, tile(q)], g32.at[q].bitcast(BF16)) for q in range(4)])
    ld_wd = copy((wd_hbm, wd_v))
    ld_w = copy(*[(w.at[0:256, tile(k)], w32.at[part, k].bitcast(BF16))
                  for part, w in enumerate((wr_hbm, wi_hbm)) for k in range(R)],
                (wr_hbm.at[256:DF], wn_v.at[0]), (wi_hbm.at[256:DF], wn_v.at[1]))
    ld_wgu = copy((wg_hbm, wg_v), (wu_hbm, wu_v))
    st_out = copy(*[(x32.at[q].bitcast(BF16), out_hbm.at[:, tile(q)]) for q in range(4)])
    st_dx = copy(*[(g32.at[q].bitcast(BF16), dx_hbm.at[:, tile(q)]) for q in range(4)])
    st_dw = copy(*[(w32.at[part, k].bitcast(BF16), w.at[0:256, tile(k)])
                   for part, w in enumerate((dwr_hbm, dwi_hbm)) for k in range(R)],
                 (dwn_v.at[0], dwr_hbm.at[256:DF]), (dwn_v.at[1], dwi_hbm.at[256:DF]))
    st_dwm = copy((wm_v, dwm_hbm))
    st_dwgu = copy((wg_v, dwg_hbm), (wu_v, dwu_hbm))
    dwgu_sem = sem.at[len(groups) - 1]
    st_dwd = copy((wd_v, dwd_hbm))

    first_row = lambda n=8: jax.lax.broadcasted_iota(jnp.int32, (n, 128), 0) == 0
    pair_rows = lambda p: pl.ds(p, N2, stride=R // 2)
    load_pairs = lambda ref, p: jnp.concatenate([ref[q, pair_rows(p), :] for q in range(4)], axis=1)

    def store_pairs(ref, p, u):
        for q in range(4):
            ref[q, pair_rows(p), :] = u[:, tile(q)]

    c = c_ref[...].astype(F32)
    sig = jax.nn.sigmoid(c)
    silu = (c * sig).astype(BF16)

    def modulate(j, n):
        mod_v[:, col(j, n)] = _dot(jnp.broadcast_to(silu, (16, D)), wm_v[:, col(j, n)])[0:8]

    mod = lambda j: mod_v[0:1, col(j)]

    def accum(j, v):
        acc_v[:, j * D:(j + 1) * D] += _colsum8(v)

    def layernorm(layer, half, p, x):
        mean = _mean(x)
        xc = x - mean
        rstd = jax.lax.rsqrt(_mean(xc * xc) + EPS)
        for k, v in enumerate((mean, rstd)):
            stat_v[2 * layer + k, half, _ds(N2 * p, N2), :] = jnp.broadcast_to(v, (N2, 128))
        return xc * rstd

    def layernorm_again(layer, half, p, x):
        mean, rstd = (_wide(stat_v[2 * layer + k, half, _ds(N2 * p, N2), :]) for k in range(2))
        return (x - mean) * rstd, rstd

    def spectral_in(p, half, h):
        h0, h1, h2, h3 = (h[:, tile(q)] for q in range(4))
        s02, s13 = h0 + h2, h1 + h3
        yee = _dot_nt(ce_ref[0], (s02 + s13).astype(BF16))
        y_v[p, 0:64, tile(half)] = yee[0:64]
        y_v[p, 64:128, tile(half)] = jnp.concatenate([jnp.where(first_row(), 0.0, yee[64:72]), yee[72:128]], axis=0)
        y_v[p, D:D + 16, tile(half)] = jnp.where(first_row(16), yee[64:80], 0.0)
        y_v[p, 128:256, tile(half)] = _dot_nt(ce_ref[1], (s02 - s13).astype(BF16))
        y_v[p, 256:D, tile(half)] = _dot_nt(co_ref[...], jnp.concatenate([h0 - h2, h1 - h3], axis=1).astype(BF16))

    def spectral_out(p, half):
        pee, peo = _dot_tn(u_v[p, 0:128, tile(half)], ce_ref[2]), _dot_tn(u_v[p, 128:256, tile(half)], ce_ref[1])
        po = _dot_tn(u_v[p, 256:D, tile(half)], co_ref[...])
        s, d = pee + peo, pee - peo
        return jnp.concatenate([s + po[:, 0:128], d + po[:, 128:256],
                                s - po[:, 0:128], d - po[:, 128:256]], axis=1)

    def filter_rows(t, w, slot, backward):
        z = _dft16([(v[:, 0:128], v[:, 128:256]) for v in t], False)
        y, dw = [], []
        for k1 in range(R):
            (zr, zi), (wr, wi) = z[k1], w(k1)
            if backward:
                xr, xi = xs_v[k1, slot, 0:128], xs_v[k1, slot, 128:256]
                dw.append((zr * xr + zi * xi, zi * xr - zr * xi))
                y.append((zr * wr + zi * wi, zi * wr - zr * wi))
            else:
                xs_v[k1, slot, 0:128] = zr
                xs_v[k1, slot, 128:256] = zi
                y.append((zr * wr - zi * wi, zr * wi + zi * wr))
        return [jnp.concatenate(v, axis=1) for v in _dft16(y, True)], dw

    def spectral_filter(backward, extra=lambda i: None):
        q = MB // 4

        def pieces(b, part):
            return (slice(64 * part + q * b, 64 * part + q * b + q),
                    slice(128 + 64 * part + q * b, 128 + 64 * part + q * b + q),
                    slice(256 + 128 * part + 2 * q * b, 256 + 128 * part + 2 * q * b + 2 * q))

        def forward(b, p, half):
            n1 = 2 * p + half
            parts = [[y_v[p, rows, tile(half)] for rows in pieces(b, part)] for part in range(2)]
            if b == 0:
                parts[0].append(y_v[p, D:D + 16, tile(half)])
                parts[1].append(jnp.zeros((16, 128), BF16))
            t = _dot(jnp.concatenate([jnp.concatenate(v, axis=0) for v in parts], axis=1), ms_v[n1])
            rows = MB + 8 * (b == 0)
            t_v[b % 2, n1, 0:rows] = t[0:rows]

        def inverse(b, n1, y):
            u = _dot_nt(y, ms_v[n1])
            for part in range(2):
                ee, eo, od = u[0:q, tile(part)], u[q:2 * q, tile(part)], u[2 * q:MB, tile(part)]
                if b == 0 and part == 1:
                    ee = jnp.concatenate([jnp.where(first_row(), u[MB:MB + 8, 0:128], ee[0:8]), ee[8:q]], axis=0)
                for rows, v in zip(pieces(b, part), (ee, eo, od)):
                    u_v[n1 // 2, rows, tile(n1 % 2)] = v

        zero = zero_ref[0]
        chunk = lambda b, k: [t_v[b % 2 + zero, n1, 8 * k:8 * k + 8] for n1 in range(R)]
        blocks, share = 256 // MB, R // (MB // 8)
        def first(i, carry):
            for k in range(4):
                forward(0, 2 * i + k // 2, k % 2)
            extra(i)
        jax.lax.fori_loop(0, R // 4, first, None)
        y = None
        for b in range(blocks):
            out = [None] * (MB // 8)
            for c in range(MB // 16):
                words = pl.ds(MB // 2 * b + 16 * (c % (q // 8)) + c // (q // 8), 8, stride=2)
                dws = []
                for odd in range(2):
                    k = c + odd * (MB // 16)
                    t = chunk(b, k)
                    for n1 in range(share * (2 * c + odd), share * (2 * c + odd + 1)):
                        if b + 1 < blocks:
                            forward(b + 1, n1 // 2, n1 % 2)
                        if b > 0:
                            inverse(b - 1, n1, y[n1])
                    w = lambda k1: tuple(_unpack(w32[part, k1, words, :])[odd] for part in range(2))
                    out[k], dw = filter_rows(t, w, slice(MB * b + 8 * k, MB * b + 8 * k + 8), backward)
                    t_v[1, 0, MB:MB + 8, 0:128] = out[k][TOKEN][:, 0:128]
                    dws.append(dw)
                if backward:
                    weight = jnp.where(first_row(), 0.5, 1.0)
                    for k1 in range(R):
                        for part in range(2):
                            lo, hi = dws[0][k1][part], dws[1][k1][part]
                            w32[part, k1, words, :] = _pack(weight * lo if b == 0 and c == 0 else lo, hi)
            if b == 0:
                w = lambda k1: tuple(jnp.broadcast_to(wn_v[part, :, tile(k1)].astype(F32), (8, 128))
                                     for part in range(2))
                last, dw = filter_rows(chunk(0, MB // 8), w, slice(256, 264), backward)
                out += [last, [jnp.zeros((8, 256), F32)] * R]
                if backward:
                    for part in range(2):
                        dwn_v[part] = (0.5 * jnp.concatenate([v[part][0:1] for v in dw], axis=1)).astype(BF16)
            y = [jnp.concatenate(v, axis=0).astype(BF16) for v in zip(*out)]
            yield
        for n1 in range(R):
            inverse(blocks - 1, n1, y[n1])

    def fwd_stats(p):
        u = load_pairs(x32, p)
        xp_v[p] = u
        for half, xf in enumerate(_unpack(u)):
            layernorm(0, half, p, xf)
        yield

    def fwd_in(p):
        for half, xf in enumerate(_unpack(xp_v[p])):
            xhat, _ = layernorm_again(0, half, p, xf)
            spectral_in(p, half, xhat * (1.0 + mod(1)) + mod(0))
            yield

    def prep_wd(i):
        quad = [wd_v[_ds(FH * a + 128 * i, 128), DH * b:DH * b + DH].astype(F32)
                for a in range(2) for b in range(2)]
        for r, v in enumerate(_rhs(*quad)):
            wd_s[r, (i, 128)] = v
        yield

    def prep_wgu(i):
        quad = [w[_ds(DH * a + 32 * i, 32), :].astype(F32) for a in range(2) for w in (wg_v, wu_v)]
        quad[1], quad[3] = 0.5 * quad[1], 0.5 * quad[3]
        for r, v in enumerate(_rhs(*quad)):
            wgu_s[r, (i, 32)] = v
        yield

    def prep_dy(p):
        rows = _ds(N2 * p, N2)
        u = load_pairs(g32, p)
        gp_v[p] = u
        top, bot = (v * mod(5) for v in _unpack(u))
        quad = (top[:, 0:DH], top[:, DH:D], bot[:, 0:DH], bot[:, DH:D])
        for r, v in enumerate(_out_t(*quad)):
            dy_s[r, (p, N2)] = v
        for r, v in enumerate(_out_t(*[t.T for t in quad])):
            dyt_s[r, :, rows] = v
        yield

    def ffn_da(p):
        for j in range(FH // 128):
            quad = _lhs_t([_dot_nt(dy_s[r, (p, N2)], wd_s[r, (j, 128)]) for r in range(7)])
            for k in range(4):
                da_v[k, (p, N2), tile(j)] = quad[k]
            yield

    def fwd_out(p):
        rows = _ds(N2 * p, N2)
        h = []
        for half, xf in enumerate(_unpack(xp_v[p])):
            y1 = spectral_out(p, half)
            yield
            y1_v[half, rows, :] = y1
            x2 = xf + (SCALE * mod(2)) * y1
            x2_v[half, rows, :] = x2
            xhat = layernorm(1, half, p, x2)
            h.append(xhat * (1.0 + mod(4)) + mod(3))
        quad = (h[0][:, 0:DH], h[0][:, DH:D], h[1][:, 0:DH], h[1][:, DH:D])
        for r, v in enumerate(_lhs(*quad)):
            h_s[r, (p, N2)] = v
        for r, v in enumerate(_lhs(*[t.T for t in quad])):
            ht_s[r, :, rows] = v
        yield

    def geglu(g, uh, da):
        g2 = g * g
        m = _G1 * g2
        t = jnp.tanh(g * (_G0 + m))
        w = 1.0 + t
        gw = g * w
        z = w + (gw * (1.0 - t)) * (_G0 + 3.0 * m)
        return gw * uh, (da * uh) * z, da * gw

    def ffn_up(i, j):
        rows, cols = (i, TP), _ds(128 * j, 128)
        a = [None] * 4
        for fh in range(2):
            fcols = _ds(FH * fh + 128 * j, 128)
            m = [_dot(h_s[r, rows], wgu_s[r, :, fcols]) for r in range(7)]
            yield
            gt, ut, gb, ub = _out(m)
            a[fh], dgt, dut = geglu(gt, ut, da_v[fh, rows, cols].astype(F32))
            a[2 + fh], dgb, dub = geglu(gb, ub, da_v[2 + fh, rows, cols].astype(F32))
            for r, v in enumerate(_out_t(dgt, dut, dgb, dub)):
                dgu_s[r, rows, fcols] = v
        for r, v in enumerate(_lhs(*a)):
            a_s[r, rows, cols] = v
        yield

    def ffn_down(p, res):
        y2, dh = [], []
        for r in range(7):
            y2.append(_dot(a_s[r, (p, N2)], wd_s[r]))
            dh.append(_dot_nt(dgu_s[r, (p, N2)], wgu_s[r]))
            yield
        res += [_out(y2), _lhs_t(dh)]

    def ffn_tail(p, res):
        rows = _ds(N2 * p, N2)
        outs = []
        for half, gout in enumerate(_unpack(gp_v[p])):
            y2, dh2 = (jnp.concatenate(v[2 * half:2 * half + 2], axis=1) for v in res)
            x2 = x2_v[half, rows, :]
            outs.append(x2 + mod(5) * y2)
            accum(5, gout * y2)
            xhat, rstd = layernorm_again(1, half, p, x2)
            accum(3, dh2)
            accum(4, dh2 * xhat)
            dx2 = gout + _layernorm_bwd(dh2 * (1.0 + mod(4)), xhat, rstd)
            accum(2, dx2 * y1_v[half, rows, :])
            x2_v[half, rows, :] = dx2
            yield
            spectral_in(p, half, dx2 * (SCALE * mod(2)))
            yield
        store_pairs(x32, p, _pack(*outs))

    def bwd_out(p):
        dx = []
        for half, xf in enumerate(_unpack(xp_v[p])):
            dh1 = spectral_out(p, half)
            yield
            xhat, rstd = layernorm_again(0, half, p, xf)
            accum(0, dh1)
            accum(1, dh1 * xhat)
            dx.append(x2_v[half, _ds(N2 * p, N2), :] + _layernorm_bwd(dh1 * (1.0 + mod(1)), xhat, rstd))
        store_pairs(g32, p, _pack(*dx))
        yield

    def mod_grads(j, n):
        dmod = jnp.sum(acc_v[:, col(j, n)], axis=0, keepdims=True)
        mod_v[:, col(j)] = _dot_nt(jnp.broadcast_to(dmod.astype(BF16), (16, n * D)), wm_v[:, col(j, n)])[0:8]
        silu_col = jnp.broadcast_to(silu.astype(F32), (128, D)).T
        for k in range(n * D // 128):
            wm_v[:, tile(j * D // 128 + k)] = (silu_col * dmod[:, tile(k)]).astype(BF16)
        yield

    def dw_down(j):
        m = []
        for r in range(7):
            m.append(_dot(dyt_s[r], a_s[r, :, _ds(128 * j, 128)]))
            yield
        for k, v in enumerate(_rhs_t(m)):
            wd_v[_ds(FH * (k // 2) + 128 * j, 128), DH * (k % 2):DH * (k % 2) + DH] = v.T.astype(BF16)
        yield

    def dw_gate_up(j):
        m = []
        for r in range(7):
            m.append(_dot(ht_s[r], dgu_s[r, :, _ds(128 * j, 128)]))
            yield
        for k, (w, v) in enumerate(zip((wg_v, wu_v, wg_v, wu_v), _rhs_t(m))):
            w[DH * (k // 2):DH * (k // 2) + DH, _ds(128 * j, 128)] = (0.5 * v if k % 2 else v).astype(BF16)
        for w, dst in ((wg_v, dwg_hbm), (wu_v, dwu_hbm)):
            cols = _ds(128 * j, 128)
            pltpu.make_async_copy(w.at[:, cols], dst.at[:, cols], dwgu_sem).start()
        yield

    def prep_dft(n1):
        fr, fi = ft_ref[0:N2, 0:128], ft_ref[0:N2, 128:256]
        tr, ti = (ft_ref[_ds(N2 + 8 * n1, 8), tile(part)][0:1] for part in range(2))
        mr, mi = fr * tr - fi * ti, fr * ti + fi * tr
        ms_v[n1, (0, N2), 0:128] = ms_v[n1, (1, N2), 128:256] = mr
        ms_v[n1, (0, N2), 128:256] = mi
        ms_v[n1, (1, N2), 0:128] = -mi
        yield

    with jax.named_scope("init"):
        start(ld_x, ld_wm0, ld_w, ld_wm5, ld_wd, ld_g, ld_wm2, ld_wgu)
        acc_v[...] = jnp.zeros(acc_v.shape, F32)
        jax.lax.fori_loop(0, R, lambda n1, carry: next(prep_dft(n1), None), None)
        wait(ld_x)
    def chain(stage, chunks, first, count):
        return (None for k in range(count) for _ in stage(first + k)), chunks * count

    _loop("stats", 0, 8, lambda p: [(fwd_stats(p), 1)])
    wait(ld_wm0)
    modulate(0, 2)
    _loop("in0", 0, 4, lambda i: [chain(fwd_in, 2, 2 * i, 2)])
    wait(ld_wm5, ld_wd, ld_w)
    modulate(5, 1)

    def fwd_filter():
        yield from spectral_filter(
            False, lambda i: _weave(chain(lambda j: prep_wd(jnp.minimum(j, FH // 128 - 1)), 1, 2 * i, 2)))
        wait(ld_g)
        yield from prep_dy(0)
    _once("filter", (fwd_filter(), 1 + 256 // MB))
    wait(ld_wm2, ld_wgu)
    modulate(2, 3)
    _loop("out", 0, R // 2, lambda p: [(ffn_da(p), 7), (fwd_out(p), 3), (prep_wgu(p), 1),
                                       (prep_dy(jnp.minimum(p + 1, R // 2 - 1)), 1)])

    def ffn(i, carry):
        _once("up", chain(lambda j: ffn_up(i, j), 3, 0, 7))
        r0, r1 = [], []
        def both():
            yield from ffn_down(2 * i, r0)
            _weave((ffn_down(2 * i + 1, r1), 7), (ffn_tail(2 * i, r0), 4))
            yield from ffn_tail(2 * i + 1, r1)
        _once("down", (both(), 11))
        return carry
    jax.lax.fori_loop(0, P // TP, ffn, 0)
    start(st_out)
    _once("bfilter", (spectral_filter(True), 256 // MB))
    start(st_dw)
    _loop("bout", 0, 4, lambda i: [chain(dw_down, 8, i, 1), chain(bwd_out, 3, 2 * i, 2)])
    start(st_dx)
    acc_v[:, col(2)] = SCALE * acc_v[:, col(2)]
    _once("dmod", chain(dw_down, 8, 4, 3), (mod_grads(0, 3), 1), (mod_grads(3, 3), 1))
    dsilu = mod_v[0:1, col(0)] + mod_v[0:1, col(3)]
    dc_ref[...] = (dsilu * (sig * (1.0 + c * (1.0 - sig)))).astype(BF16)
    start(st_dwm, st_dwd)
    _loop("dwgu", 0, F // 256, lambda j: [chain(dw_gate_up, 8, 2 * j, 2)])
    with jax.named_scope("drain"):
        wait(st_out, st_dw, st_dx, st_dwm, st_dwd, st_dwgu)


@jax.jit
def pallas_adaLN_cond__spectral_gfnet__geglu_ffn__prompt_kernel(
    A_x: jax.Array,
    A_w_r: jax.Array,
    A_w_i: jax.Array,
    B_x: jax.Array,
    B_w_gate: jax.Array,
    B_w_up: jax.Array,
    B_w_down: jax.Array,
    c: jax.Array,
    w_mod: jax.Array,
    grad_out: jax.Array,
):
    del B_x
    hbm = pl.BlockSpec(memory_space=pltpu.HBM)
    vmem = pl.BlockSpec(memory_space=pltpu.VMEM)
    sds = lambda *s: jax.ShapeDtypeStruct(s, BF16)
    v = pltpu.VMEM
    pk = lambda n, rows, cols: v((n, rows // 2, cols), U32)
    outs = pl.pallas_call(
        _kernel,
        in_specs=[hbm] * 6 + [vmem] + [hbm] * 2 + [vmem] * 3 + [pl.BlockSpec(memory_space=pltpu.SMEM)],
        out_specs=[hbm] * 7 + [vmem, hbm],
        out_shape=[sds(S, D), sds(S, D), sds(DF, S), sds(DF, S), sds(D, F), sds(D, F), sds(F, D),
                   sds(1, D), sds(D, 6 * D)],
        scratch_shapes=[
            v((4, P, 128), U32), v((4, P, 128), U32),
            v((2, R, 128, 128), U32), v((2, 1, S), BF16),
            v((D, F), BF16), v((D, F), BF16), v((F, D), BF16), v((D, 6 * D), BF16),
            pk(R, 256, 256),
            v((R // 2, N2, D), U32), v((R // 2, N2, D), U32),
            pk(R // 2, D + 16, 256), pk(R // 2, D, 256), v((R, 264, 256), F32),
            v((2, P, D), F32), v((2, P, D), F32),
            pk(7, DH, F), pk(7, FH, DH),
            pk(7, P, DH), pk(7, DH, P),
            pk(7, P, DH), pk(7, DH, P),
            pk(4, P, FH), pk(7, P, FH), pk(7, P, F),
            v((8, 6 * D), F32), v((8, 6 * D), F32),
            v((2, 1, S), BF16),
            v((4, 2, P, 128), F32), v((2, R, MB + 8, 256), F32),
            pltpu.SemaphoreType.DMA((24,)),
        ],
        compiler_params=pltpu.CompilerParams(vmem_limit_bytes=127 * 1024 * 1024),
    )(A_x.reshape(S, D), A_w_r.T, A_w_i.T, B_w_gate, B_w_up, B_w_down, c, w_mod,
      grad_out.reshape(S, D), _CE, _CO, _FT, np.zeros((1,), np.int32))
    return (outs[0].reshape(1, S, D), outs[1].reshape(1, S, D), outs[2].T, outs[3].T, *outs[4:])
```

```python
import numpy as np
import jax
import jax.numpy as jnp
import jax.experimental.pallas as pl
import jax.experimental.pallas.tpu as pltpu

S, D, F = 2048, 512, 1792
DF = D // 2 + 1
R, N2 = 16, 128
P = S // 2
SCALE = 2.0 / (S * D)
DH, FH = D // 2, F // 2
XC = 512
EPS = 1e-5
F32, BF16, U32 = jnp.float32, jnp.bfloat16, jnp.uint32
TP = 256

_G0 = float(np.sqrt(2.0 / np.pi))
_G1 = _G0 * 0.044715


def _constants():
    def dft(m, n):
        ang = 2 * np.pi * ((m[:, None] * np.arange(n)[None, :]) % D) / D
        return np.concatenate([np.cos(ang), -np.sin(ang)], axis=0)
    i = np.arange(64)
    cee, ceo = dft(4 * i, 128), dft(4 * i + 2, 128)
    cee[64] = 1.0 - 2.0 * (np.arange(128) % 2)
    j = np.arange(128)
    co = dft(4 * (j % 64) + 1 + 2 * (j // 64), 256)
    weight = np.ones((128, 1))
    weight[0] = weight[64] = 0.5
    ce = np.stack([cee, ceo, weight * cee])
    k2 = np.arange(N2)[None, :]
    ang = 2 * np.pi * np.concatenate([(np.arange(N2)[:, None] * k2 % N2) / N2, np.arange(8 * R)[:, None] // 8 * k2 / S])
    ft = np.concatenate([np.cos(ang), -np.sin(ang)], axis=1).astype(np.float32)
    return ce.astype(jnp.bfloat16), co.astype(jnp.bfloat16), ft


_CE, _CO, _FT = _constants()


def _dft4(x, inv):
    (ar, ai), (br, bi), (cr, ci), (dr, di) = x
    s0r, s0i, d0r, d0i = ar + cr, ai + ci, ar - cr, ai - ci
    s1r, s1i, d1r, d1i = br + dr, bi + di, br - dr, bi - di
    p = (d0r + d1i, d0i - d1r)
    q = (d0r - d1i, d0i + d1r)
    return [(s0r + s1r, s0i + s1i), q if inv else p, (s0r - s1r, s0i - s1i), p if inv else q]


def _twiddle16(v, e, inv):
    r, i = v
    if e == 0:
        return v
    h = float(np.sqrt(0.5))
    if e == 4:
        return (-i, r) if inv else (i, -r)
    if e == 2:
        return ((r - i) * h, (r + i) * h) if inv else ((r + i) * h, (i - r) * h)
    if e == 6:
        return ((r + i) * (-h), (r - i) * h) if inv else ((i - r) * h, (r + i) * (-h))
    c = float(np.cos(2 * np.pi * e / 16))
    s = float(np.sin(2 * np.pi * e / 16)) * (1.0 if inv else -1.0)
    return (r * c - i * s, r * s + i * c)


def _dft16(x, inv):
    t = [_dft4([x[4 * a + b] for a in range(4)], inv) for b in range(4)]
    out = [None] * 16
    for c in range(4):
        col = _dft4([_twiddle16(t[b][c], b * c, inv) for b in range(4)], inv)
        for d in range(4):
            out[c + 4 * d] = col[d]
    return out


def _dot(a, b):
    return jnp.dot(a, b, preferred_element_type=F32)


def _mean(v):
    return jnp.sum(v, axis=-1, keepdims=True) * (1.0 / D)


def _colsum8(v):
    return jnp.sum(v.reshape(v.shape[0] // 8, 8, v.shape[1]), axis=0)


def _wide(v):
    return jnp.concatenate([v] * (D // 128), axis=1)


def _layernorm_bwd(dxhat, xhat, rstd):
    return rstd * (dxhat - _mean(dxhat) - xhat * _mean(dxhat * xhat))


def _ds(start, size):
    return pl.ds(start if isinstance(start, int) else pl.multiple_of(start, size), size)


class _Packed:
    def __init__(self, ref):
        self.ref = ref

    @staticmethod
    def _index(idx, packing):
        lead, rows, cols = (idx + (slice(None),))[:3] if isinstance(idx, tuple) else (idx, slice(None), slice(None))
        if isinstance(rows, tuple):
            rows = _ds(rows[0] * (rows[1] // packing), rows[1] // packing)
        elif rows != slice(None):
            rows = slice(rows.start // packing, rows.stop // packing)
        return lead, rows, cols

    def __getitem__(self, idx):
        return pltpu.bitcast(self.ref[self._index(idx, 2)], BF16)

    def __setitem__(self, idx, value):
        lead, rows, cols = self._index(idx, 1)
        self.ref.at[lead].bitcast(BF16)[rows, cols] = value.astype(BF16)


def _loop(name, lo, hi, streams):
    def body(i, carry):
        _weave(*streams(i))
        return carry
    with jax.named_scope(name):
        jax.lax.fori_loop(lo, hi, body, 0)


def _once(name, *streams):
    with jax.named_scope(name):
        _weave(*streams)


def _weave(*streams):
    steps = sorted(((k + 0.5) / n, s) for s, (_, n) in enumerate(streams) for k in range(n))
    for _, s in steps:
        next(streams[s][0])
    for gen, _ in streams:
        assert next(gen, 1) == 1


def _dot_nt(a, b):
    return jax.lax.dot_general(a, b, (((1,), (1,)), ((), ())), preferred_element_type=F32)


def _dot_tn(a, b):
    return jax.lax.dot_general(a, b, (((0,), (0,)), ((), ())), preferred_element_type=F32)


def _unpack(u):
    return pltpu.bitcast(u << 16, F32), pltpu.bitcast(u & jnp.uint32(0xFFFF0000), F32)


def _pack(lo, hi):
    lo = pltpu.bitcast(lo.astype(BF16).astype(F32), U32) >> 16
    return lo | pltpu.bitcast(hi.astype(BF16).astype(F32), U32)


def _lhs(a11, a12, a21, a22):
    return [a11 + a22, a21 + a22, a11, a22, a11 + a12, a21 - a11, a12 - a22]


def _rhs(b11, b12, b21, b22):
    return [b11 + b22, b11, b12 - b22, b21 - b11, b22, b11 + b12, b21 + b22]


def _out(m):
    return m[0] + m[3] - m[4] + m[6], m[2] + m[4], m[1] + m[3], m[0] - m[1] + m[2] + m[5]


def _out_t(c11, c12, c21, c22):
    return [c11 + c22, c21 - c22, c12 + c22, c11 + c21, c12 - c11, c22, c11]


def _lhs_t(m):
    return m[0] + m[2] + m[4] - m[5], m[4] + m[6], m[1] + m[5], m[0] + m[1] + m[3] - m[6]


def _rhs_t(m):
    return m[0] + m[1] - m[3] + m[5], m[2] + m[5], m[3] + m[6], m[0] - m[2] + m[4] + m[6]


def _kernel(x_hbm, wr_hbm, wi_hbm, wg_hbm, wu_hbm, wd_hbm, c_ref, wm_hbm, g_hbm,
            ce_ref, co_ref, ft_ref,
            out_hbm, dx_hbm, dwr_hbm, dwi_hbm, dwg_hbm, dwu_hbm, dwd_hbm, dc_ref, dwm_hbm,
            x32, g32, w32, wn_v, wg_v, wu_v, wd_v, wm_v, ms_v,
            xp_v, gp_v, y_v, v_v, u_v, xs_v, y1_v, x2_v,
            wgu_s, wd_s, h_s, ht_s, dy_s, dyt_s, da_v, a_s, dgu_s,
            mod_v, acc_v, dwn_v, stat_v, t_v, sem):
    (ms_v, y_v, v_v, u_v, wgu_s, wd_s, h_s, ht_s, dy_s, dyt_s, da_v, a_s, dgu_s) = map(_Packed, (
        ms_v, y_v, v_v, u_v, wgu_s, wd_s, h_s, ht_s, dy_s, dyt_s, da_v, a_s, dgu_s))
    groups = []

    def copy(*pairs):
        group = [pltpu.make_async_copy(src, dst, sem.at[len(groups)]) for src, dst in pairs]
        groups.append(group)
        return group

    def start(*new):
        for group in new:
            for cp in group:
                cp.start()

    def wait(*started):
        for group in started:
            for cp in group:
                cp.wait()

    tile = lambda q: slice(128 * q, 128 * q + 128)
    col = lambda j, n=1: slice(D * j, D * (j + n))
    ld_wm = lambda j, n: copy((wm_hbm.at[:, col(j, n)], wm_v.at[:, col(j, n)]))
    ld_wm0, ld_wm2 = ld_wm(0, 2), ld_wm(2, 4)
    ld_x = [copy(*[(x_hbm.at[XC * k:XC * k + XC, tile(q)], x32.at[q, XC // 2 * k:XC // 2 * (k + 1)].bitcast(BF16))
                   for q in range(4)]) for k in range(S // XC)]
    ld_g = copy(*[(g_hbm.at[:, tile(q)], g32.at[q].bitcast(BF16)) for q in range(4)])
    ld_wd = copy((wd_hbm, wd_v))
    ld_w = copy(*[(w.at[0:256, tile(k)], w32.at[part, k].bitcast(BF16))
                  for part, w in enumerate((wr_hbm, wi_hbm)) for k in range(R)],
                (wr_hbm.at[256:DF], wn_v.at[0]), (wi_hbm.at[256:DF], wn_v.at[1]))
    ld_wgu = copy((wg_hbm, wg_v), (wu_hbm, wu_v))
    st_out = copy(*[(x32.at[q].bitcast(BF16), out_hbm.at[:, tile(q)]) for q in range(4)])
    st_dx = copy(*[(g32.at[q].bitcast(BF16), dx_hbm.at[:, tile(q)]) for q in range(4)])
    st_dw = copy(*[(w32.at[part, k].bitcast(BF16), w.at[0:256, tile(k)])
                   for part, w in enumerate((dwr_hbm, dwi_hbm)) for k in range(R)],
                 (dwn_v.at[0], dwr_hbm.at[256:DF]), (dwn_v.at[1], dwi_hbm.at[256:DF]))
    st_dwm = copy((wm_v, dwm_hbm))
    st_dwgu = copy((wg_v, dwg_hbm), (wu_v, dwu_hbm))
    dwgu_sem = sem.at[len(groups) - 1]
    st_dwd = copy((wd_v, dwd_hbm))

    first_row = lambda n=8: jax.lax.broadcasted_iota(jnp.int32, (n, 128), 0) == 0
    pair_rows = lambda p: pl.ds(p, N2, stride=R // 2)
    load_pairs = lambda ref, p: jnp.concatenate([ref[q, pair_rows(p), :] for q in range(4)], axis=1)

    def store_pairs(ref, p, u):
        for q in range(4):
            ref[q, pair_rows(p), :] = u[:, tile(q)]

    def silu():
        c = c_ref[...].astype(F32)
        sig = jax.nn.sigmoid(c)
        return (c * sig).astype(BF16), sig * (1.0 + c * (1.0 - sig))

    def modulate(j, n):
        mod_v[:, col(j, n)] = _dot(jnp.broadcast_to(silu()[0], (16, D)), wm_v[:, col(j, n)])[0:8]

    mod = lambda j: mod_v[0:1, col(j)]

    def accum(j, v):
        acc_v[:, j * D:(j + 1) * D] += _colsum8(v)

    def layernorm(layer, half, rows, x):
        mean = _mean(x)
        xc = x - mean
        rstd = jax.lax.rsqrt(_mean(xc * xc) + EPS)
        for k, v in enumerate((mean, rstd)):
            stat_v[2 * layer + k, half, rows, :] = jnp.broadcast_to(v, (x.shape[0], 128))
        return xc * rstd

    def layernorm_again(layer, half, rows, x):
        mean, rstd = (_wide(stat_v[2 * layer + k, half, rows, :]) for k in range(2))
        return (x - mean) * rstd, rstd

    def spectral_in(p, half, h):
        h0, h1, h2, h3 = (h[:, tile(q)] for q in range(4))
        s02, s13 = h0 + h2, h1 + h3
        yee = _dot_nt(ce_ref[0], (s02 + s13).astype(BF16))
        yeo = _dot_nt(ce_ref[1], (s02 - s13).astype(BF16))
        yo = _dot_nt(co_ref[...], jnp.concatenate([h0 - h2, h1 - h3], axis=1).astype(BF16))
        re = jnp.concatenate([yee[0:64], yeo[0:64], yo[0:128]], axis=0)
        im = jnp.concatenate([jnp.where(first_row(), 0.0, yee[64:72]), yee[72:128], yeo[64:128], yo[128:256]], axis=0)
        for k, v in enumerate((re, im, re + im)):
            y_v[p, 256 * k:256 * k + 256, tile(half)] = v
        y_v[p, 768:784, tile(half)] = jnp.where(first_row(16), yee[64:80], 0.0)

    def spectral_out(p, half):
        pee, peo = _dot_tn(u_v[p, 0:128, tile(half)], ce_ref[2]), _dot_tn(u_v[p, 128:256, tile(half)], ce_ref[1])
        po = _dot_tn(u_v[p, 256:D, tile(half)], co_ref[...])
        s, d = pee + peo, pee - peo
        return jnp.concatenate([s + po[:, 0:128], d + po[:, 128:256],
                                s - po[:, 0:128], d - po[:, 128:256]], axis=1)

    def filter_rows(t, w, slot, backward):
        z = _dft16([(v[:, 0:128], v[:, 128:256]) for v in t], False)
        y, dw = [], []
        for k1 in range(R):
            (zr, zi), (wr, wi) = z[k1], w(k1)
            if backward:
                xr, xi = xs_v[k1, slot, 0:128], xs_v[k1, slot, 128:256]
                dw.append((zr * xr + zi * xi, zi * xr - zr * xi))
                y.append((zr * wr + zi * wi, zi * wr - zr * wi))
            else:
                xs_v[k1, slot, 0:128] = zr
                xs_v[k1, slot, 128:256] = zi
                y.append((zr * wr - zi * wi, zr * wi + zi * wr))
        return _dft16(y, True), dw

    def tokens_fwd(p):
        for half in range(2):
            n1, last = 2 * p + half, y_v[p, 768:784, tile(half)]
            re, im, both = (jnp.concatenate([y_v[p, 256 * k:256 * k + 256, tile(half)], w], axis=0)
                            for k, w in enumerate((last, jnp.zeros_like(last), last)))
            k = _dot(both, ms_v[n1, :, 0:128])
            t_v[n1, :, 0:128] = (k - _dot(im, ms_v[n1, :, 128:256]))[0:264]
            t_v[n1, :, 128:256] = (k + _dot(re, ms_v[n1, :, 256:384]))[0:264]
            yield

    def tokens_inv(p):
        for half in range(2):
            n1 = 2 * p + half
            k = _dot_nt(v_v[n1, :, tile(2)], ms_v[n1, :, 0:128])
            u = (k + _dot_nt(v_v[n1, :, tile(1)], ms_v[n1, :, 256:384]),
                 k - _dot_nt(v_v[n1, :, tile(0)], ms_v[n1, :, 128:256]))
            even, odd = ([[v[16 * c + 8 * j:16 * c + 8 * j + 8] for c in range(16)] for v in u] for j in range(2))
            even[1][0] = jnp.where(first_row(), u[0][256:264], even[1][0])
            u_v[p, :, tile(half)] = jnp.concatenate(
                even[0][:8] + even[1][:8] + even[0][8:] + even[1][8:] + odd[0] + odd[1], axis=0)
            yield

    def keep(c, first, second):
        for n1 in range(R):
            vr, vi = (jnp.concatenate([first[n1][k], second[n1][k]], axis=0) for k in range(2))
            v_v[n1, (c, 16)] = jnp.concatenate([vr, vi, vr + vi], axis=1)

    def filter_words(c, backward):
        words = pl.ds(16 * (c % 8) + c // 8, 8, stride=2)
        ys, dws = [], []
        for odd in range(2):
            rows = _ds(128 * odd + 8 * c, 8)
            w = lambda k1: tuple(_unpack(w32[part, k1, words, :])[odd] for part in range(2))
            y, dw = filter_rows([t_v[n1, rows] for n1 in range(R)], w, rows, backward)
            t_v[0, rows, 0:128] = y[R - 1][0]
            ys.append(y)
            dws.append(dw)
        keep(c, *ys)
        if backward:
            weight = jnp.where(jax.lax.broadcasted_iota(jnp.int32, (8, 128), 0) + c == 0, 0.5, 1.0)
            for k1 in range(R):
                for part in range(2):
                    w32[part, k1, words, :] = _pack(weight * dws[0][k1][part], dws[1][k1][part])
        yield

    def filter_last(backward):
        w = lambda k1: tuple(jnp.broadcast_to(wn_v[part, :, tile(k1)].astype(F32), (8, 128)) for part in range(2))
        y, dw = filter_rows([t_v[n1, 256:264] for n1 in range(R)], w, slice(256, 264), backward)
        keep(16, y, [(jnp.zeros((8, 128), F32),) * 2] * R)
        if backward:
            for part in range(2):
                dwn_v[part] = (0.5 * jnp.concatenate([v[part][0:1] for v in dw], axis=1)).astype(BF16)
        yield

    def fwd_stats(i):
        for p in range(R // 2):
            u = jnp.concatenate([x32[q, pl.ds(N2 * i + p, 16, stride=R // 2), :] for q in range(4)], axis=1)
            xp_v[p, _ds(16 * i, 16), :] = u
            for half, xf in enumerate(_unpack(u)):
                layernorm(0, half, _ds(N2 * p + 16 * i, 16), xf)
        yield

    def fwd_in(p):
        for half, xf in enumerate(_unpack(xp_v[p])):
            xhat, _ = layernorm_again(0, half, _ds(N2 * p, N2), xf)
            spectral_in(p, half, xhat * (1.0 + mod(1)) + mod(0))
            yield

    def prep_wd(i):
        for k in range(8):
            quad = [wd_v[_ds(FH * a + 128 * i + 16 * k, 16), DH * b:DH * b + DH].astype(F32)
                    for a in range(2) for b in range(2)]
            for r, v in enumerate(_rhs(*quad)):
                wd_s[r, (8 * i + k, 16)] = v
        yield

    def prep_wgu(i):
        for k in range(2):
            for cols in (slice(lo, lo + 256) for lo in range(0, F, 256)):
                quad = [w[_ds(DH * a + 32 * i + 16 * k, 16), cols].astype(F32)
                        for a in range(2) for w in (wg_v, wu_v)]
                quad[1], quad[3] = 0.5 * quad[1], 0.5 * quad[3]
                for r, v in enumerate(_rhs(*quad)):
                    wgu_s[r, (2 * i + k, 16), cols] = v
        yield

    def prep_dy(p):
        rows = _ds(N2 * p, N2)
        u = load_pairs(g32, p)
        gp_v[p] = u
        top, bot = (v * mod(5) for v in _unpack(u))
        quad = (top[:, 0:DH], top[:, DH:D], bot[:, 0:DH], bot[:, DH:D])
        for r, v in enumerate(_out_t(*quad)):
            dy_s[r, (p, N2)] = v
        for r, v in enumerate(_out_t(*[t.T for t in quad])):
            dyt_s[r, :, rows] = v
        yield

    def ffn_da(p):
        for j in range(FH // 128):
            quad = _lhs_t([_dot_nt(dy_s[r, (p, N2)], wd_s[r, (j, 128)]) for r in range(7)])
            for k in range(4):
                da_v[k, (p, N2), tile(j)] = quad[k]
            yield

    def fwd_out(p):
        rows = _ds(N2 * p, N2)
        h = []
        for half, xf in enumerate(_unpack(xp_v[p])):
            y1 = spectral_out(p, half)
            yield
            y1_v[half, rows, :] = y1
            x2 = xf + (SCALE * mod(2)) * y1
            x2_v[half, rows, :] = x2
            xhat = layernorm(1, half, rows, x2)
            h.append(xhat * (1.0 + mod(4)) + mod(3))
        quad = (h[0][:, 0:DH], h[0][:, DH:D], h[1][:, 0:DH], h[1][:, DH:D])
        for r, v in enumerate(_lhs(*quad)):
            h_s[r, (p, N2)] = v
        for r, v in enumerate(_lhs(*[t.T for t in quad])):
            ht_s[r, :, rows] = v
        yield

    def geglu(g, uh, da):
        g2 = g * g
        m = _G1 * g2
        t = jnp.tanh(g * (_G0 + m))
        w = 1.0 + t
        gw = g * w
        z = w + (gw * (1.0 - t)) * (_G0 + 3.0 * m)
        return gw * uh, (da * uh) * z, da * gw

    def ffn_up(i, j):
        rows, cols = (i, TP), _ds(128 * j, 128)
        a = [None] * 4
        for fh in range(2):
            fcols = _ds(FH * fh + 128 * j, 128)
            m = [_dot(h_s[r, rows], wgu_s[r, :, fcols]) for r in range(7)]
            yield
            gt, ut, gb, ub = _out(m)
            a[fh], dgt, dut = geglu(gt, ut, da_v[fh, rows, cols].astype(F32))
            a[2 + fh], dgb, dub = geglu(gb, ub, da_v[2 + fh, rows, cols].astype(F32))
            for r, v in enumerate(_out_t(dgt, dut, dgb, dub)):
                dgu_s[r, rows, fcols] = v
        for r, v in enumerate(_lhs(*a)):
            a_s[r, rows, cols] = v
        yield

    def ffn_down(p, res):
        y2, dh = [], []
        for r in range(7):
            y2.append(_dot(a_s[r, (p, N2)], wd_s[r]))
            dh.append(_dot_nt(dgu_s[r, (p, N2)], wgu_s[r]))
            yield
        res += [_out(y2), _lhs_t(dh)]

    def ffn_tail(p, res):
        rows = _ds(N2 * p, N2)
        outs = []
        for half, gout in enumerate(_unpack(gp_v[p])):
            y2, dh2 = (jnp.concatenate(v[2 * half:2 * half + 2], axis=1) for v in res)
            x2 = x2_v[half, rows, :]
            outs.append(x2 + mod(5) * y2)
            accum(5, gout * y2)
            xhat, rstd = layernorm_again(1, half, rows, x2)
            accum(3, dh2)
            accum(4, dh2 * xhat)
            dx2 = gout + _layernorm_bwd(dh2 * (1.0 + mod(4)), xhat, rstd)
            accum(2, dx2 * y1_v[half, rows, :])
            x2_v[half, rows, :] = dx2
            yield
            spectral_in(p, half, dx2 * (SCALE * mod(2)))
            yield
        store_pairs(x32, p, _pack(*outs))

    def bwd_out(p):
        dx = []
        for half, xf in enumerate(_unpack(xp_v[p])):
            dh1 = spectral_out(p, half)
            yield
            xhat, rstd = layernorm_again(0, half, _ds(N2 * p, N2), xf)
            accum(0, dh1)
            accum(1, dh1 * xhat)
            dx.append(x2_v[half, _ds(N2 * p, N2), :] + _layernorm_bwd(dh1 * (1.0 + mod(1)), xhat, rstd))
        store_pairs(g32, p, _pack(*dx))
        yield

    def mod_grads(j, n):
        dmod = jnp.sum(acc_v[:, col(j, n)], axis=0, keepdims=True)
        mod_v[:, col(j)] = _dot_nt(jnp.broadcast_to(dmod.astype(BF16), (16, n * D)), wm_v[:, col(j, n)])[0:8]
        silu_col = jnp.broadcast_to(silu()[0].astype(F32), (128, D)).T
        for k in range(n * D // 128):
            wm_v[:, tile(j * D // 128 + k)] = (silu_col * dmod[:, tile(k)]).astype(BF16)
        yield

    def dw_down(j):
        m = []
        for r in range(7):
            m.append(_dot(dyt_s[r], a_s[r, :, _ds(128 * j, 128)]))
            yield
        for k, v in enumerate(_rhs_t(m)):
            wd_v[_ds(FH * (k // 2) + 128 * j, 128), DH * (k % 2):DH * (k % 2) + DH] = v.T.astype(BF16)
        yield

    def dw_gate_up(j):
        m = []
        for r in range(7):
            m.append(_dot(ht_s[r], dgu_s[r, :, _ds(128 * j, 128)]))
            yield
        for k, (w, v) in enumerate(zip((wg_v, wu_v, wg_v, wu_v), _rhs_t(m))):
            w[DH * (k // 2):DH * (k // 2) + DH, _ds(128 * j, 128)] = (0.5 * v if k % 2 else v).astype(BF16)
        for w, dst in ((wg_v, dwg_hbm), (wu_v, dwu_hbm)):
            cols = _ds(128 * j, 128)
            pltpu.make_async_copy(w.at[:, cols], dst.at[:, cols], dwgu_sem).start()
        yield

    def prep_dft(n1):
        fr, fi = ft_ref[0:N2, 0:128], ft_ref[0:N2, 128:256]
        tr, ti = (ft_ref[_ds(N2 + 8 * n1, 8), tile(part)][0:1] for part in range(2))
        mr, mi = fr * tr - fi * ti, fr * ti + fi * tr
        ms_v[n1] = jnp.concatenate([mr, mr + mi, mi - mr], axis=1)
        yield

    with jax.named_scope("init"):
        start(*ld_x, ld_wm0, ld_wd, ld_w, ld_wm2, ld_g, ld_wgu)
        acc_v[...] = jnp.zeros(acc_v.shape, F32)
        jax.lax.fori_loop(0, R, lambda n1, carry: next(prep_dft(n1), None), None)
    def chain(stage, chunks, first, count):
        return (None for k in range(count) for _ in stage(first + k)), chunks * count


    def stats(i):
        for k, group in enumerate(ld_x):
            pl.when(i == k * (XC // 2 // N2))(lambda: wait(group))
        return [(fwd_stats(i), 1)]
    _loop("stats", 0, P // N2, stats)
    wait(ld_wm0)
    modulate(0, 2)
    _loop("in0", 0, R // 4, lambda i: [chain(fwd_in, 2, 2 * i, 2)])
    wait(ld_wd)
    _loop("s_fwd", 0, R // 2, lambda p: [(tokens_fwd(p), 2), (prep_wd(jnp.minimum(p, FH // 128 - 1)), 1)])
    wait(ld_w)
    _loop("filter", 0, 16, lambda c: [(filter_words(c, False), 1)])
    _once("filter", (filter_last(False), 1))
    wait(ld_wm2, ld_g)
    modulate(2, 4)
    _loop("s_inv", 0, R // 2, lambda p: [(tokens_inv(p), 2), (prep_dy(p), 1)])
    wait(ld_wgu)
    _loop("out", 0, R // 2, lambda p: [(ffn_da(p), 7), (fwd_out(p), 3), (prep_wgu(p), 1)])

    def ffn(i, carry):
        r0, r1 = [], []
        _once("up", chain(lambda j: ffn_up(i, j), 3, 0, FH // 128))
        with jax.named_scope("down"):
            _weave((ffn_down(2 * i, r0), 7))
            _weave((ffn_down(2 * i + 1, r1), 7), (ffn_tail(2 * i, r0), 4))
            _weave((tokens_fwd(jnp.maximum(2 * i - 1, 0)), 2), (tokens_fwd(2 * i), 2))
            _weave((ffn_tail(2 * i + 1, r1), 4))
        return carry
    jax.lax.fori_loop(0, P // TP, ffn, 0)
    start(st_out)
    _once("s_fwd2", (tokens_fwd(R // 2 - 1), 2))
    _loop("bfilter", 0, 16, lambda c: [(filter_words(c, True), 1)])
    _once("bfilter", (filter_last(True), 1))
    start(st_dw)
    _once("s_inv2", chain(tokens_inv, 2, 0, 2))
    _loop("bout", 0, 3, lambda i: [chain(dw_down, 8, i, 1), chain(bwd_out, 3, 2 * i, 2),
                                   chain(tokens_inv, 2, 2 * i + 2, 2)])
    _once("bout", chain(dw_down, 8, 3, 1), chain(bwd_out, 3, 6, 2), (mod_grads(3, 3), 1))
    start(st_dx)
    acc_v[:, col(2)] = SCALE * acc_v[:, col(2)]
    _once("dmod", chain(dw_down, 8, 4, 3), (mod_grads(0, 3), 1))
    dsilu = mod_v[0:1, col(0)] + mod_v[0:1, col(3)]
    dc_ref[...] = (dsilu * silu()[1]).astype(BF16)
    start(st_dwm, st_dwd)
    _loop("dwgu", 0, F // 256, lambda j: [chain(dw_gate_up, 8, 2 * j, 2)])
    with jax.named_scope("drain"):
        wait(st_out, st_dw, st_dx, st_dwm, st_dwd, st_dwgu)


@jax.jit
def pallas_adaLN_cond__spectral_gfnet__geglu_ffn__prompt_kernel(
    A_x: jax.Array,
    A_w_r: jax.Array,
    A_w_i: jax.Array,
    B_x: jax.Array,
    B_w_gate: jax.Array,
    B_w_up: jax.Array,
    B_w_down: jax.Array,
    c: jax.Array,
    w_mod: jax.Array,
    grad_out: jax.Array,
):
    del B_x
    hbm = pl.BlockSpec(memory_space=pltpu.HBM)
    vmem = pl.BlockSpec(memory_space=pltpu.VMEM)
    sds = lambda *s: jax.ShapeDtypeStruct(s, BF16)
    v = pltpu.VMEM
    pk = lambda n, rows, cols: v((n, rows // 2, cols), U32)
    outs = pl.pallas_call(
        _kernel,
        in_specs=[hbm] * 6 + [vmem] + [hbm] * 2 + [vmem] * 3,
        out_specs=[hbm] * 7 + [vmem, hbm],
        out_shape=[sds(S, D), sds(S, D), sds(DF, S), sds(DF, S), sds(D, F), sds(D, F), sds(F, D),
                   sds(1, D), sds(D, 6 * D)],
        scratch_shapes=[
            v((4, P, 128), U32), v((4, P, 128), U32),
            v((2, R, 128, 128), U32), v((2, 1, S), BF16),
            v((D, F), BF16), v((D, F), BF16), v((F, D), BF16), v((D, 6 * D), BF16),
            pk(R, N2, 384),
            v((R // 2, N2, D), U32), v((R // 2, N2, D), U32),
            pk(R // 2, 784, 256), pk(R, 272, 384), pk(R // 2, D, 256), v((R, 264, 256), F32),
            v((2, P, D), F32), v((2, P, D), F32),
            pk(7, DH, F), pk(7, FH, DH),
            pk(7, P, DH), pk(7, DH, P),
            pk(7, P, DH), pk(7, DH, P),
            pk(4, P, FH), pk(7, P, FH), pk(7, P, F),
            v((8, 6 * D), F32), v((8, 6 * D), F32),
            v((2, 1, S), BF16),
            v((4, 2, P, 128), F32), v((R, 264, 256), F32),
            pltpu.SemaphoreType.DMA((24,)),
        ],
        compiler_params=pltpu.CompilerParams(vmem_limit_bytes=127 * 1024 * 1024),
    )(A_x.reshape(S, D), A_w_r.T, A_w_i.T, B_w_gate, B_w_up, B_w_down, c, w_mod,
      grad_out.reshape(S, D), _CE, _CO, _FT)
    return (outs[0].reshape(1, S, D), outs[1].reshape(1, S, D), outs[2].T, outs[3].T, *outs[4:])
```

```python
import numpy as np
import jax
import jax.numpy as jnp
import jax.experimental.pallas as pl
import jax.experimental.pallas.tpu as pltpu

S, D, F = 2048, 512, 1792
DF = D // 2 + 1
R, N2 = 16, 128
P = S // 2
SCALE = 2.0 / (S * D)
DH, FH = D // 2, F // 2
XC = 512
EPS = 1e-5
F32, BF16, U32 = jnp.float32, jnp.bfloat16, jnp.uint32
TP = 256

_G0 = float(np.sqrt(2.0 / np.pi))
_G1 = _G0 * 0.044715


def _constants():
    def dft(m, n):
        ang = 2 * np.pi * ((m[:, None] * np.arange(n)[None, :]) % D) / D
        return np.concatenate([np.cos(ang), -np.sin(ang)], axis=0)
    i = np.arange(64)
    cee, ceo = dft(4 * i, 128), dft(4 * i + 2, 128)
    cee[64] = 1.0 - 2.0 * (np.arange(128) % 2)
    j = np.arange(128)
    co = dft(4 * (j % 64) + 1 + 2 * (j // 64), 256)
    weight = np.ones((128, 1))
    weight[0] = weight[64] = 0.5
    ce = np.stack([cee, ceo, weight * cee])
    k2 = np.arange(N2)[None, :]
    ang = 2 * np.pi * np.concatenate([(np.arange(N2)[:, None] * k2 % N2) / N2, np.arange(8 * R)[:, None] // 8 * k2 / S])
    ft = np.concatenate([np.cos(ang), -np.sin(ang)], axis=1).astype(np.float32)
    return ce.astype(jnp.bfloat16), co.astype(jnp.bfloat16), ft


_CE, _CO, _FT = _constants()


def _dft4(x, inv):
    (ar, ai), (br, bi), (cr, ci), (dr, di) = x
    s0r, s0i, d0r, d0i = ar + cr, ai + ci, ar - cr, ai - ci
    s1r, s1i, d1r, d1i = br + dr, bi + di, br - dr, bi - di
    p = (d0r + d1i, d0i - d1r)
    q = (d0r - d1i, d0i + d1r)
    return [(s0r + s1r, s0i + s1i), q if inv else p, (s0r - s1r, s0i - s1i), p if inv else q]


def _twiddle16(v, e, inv):
    r, i = v
    if e == 0:
        return v
    h = float(np.sqrt(0.5))
    if e == 4:
        return (-i, r) if inv else (i, -r)
    if e == 2:
        return ((r - i) * h, (r + i) * h) if inv else ((r + i) * h, (i - r) * h)
    if e == 6:
        return ((r + i) * (-h), (r - i) * h) if inv else ((i - r) * h, (r + i) * (-h))
    c = float(np.cos(2 * np.pi * e / 16))
    s = float(np.sin(2 * np.pi * e / 16)) * (1.0 if inv else -1.0)
    return (r * c - i * s, r * s + i * c)


def _dft16(x, inv):
    t = [_dft4([x[4 * a + b] for a in range(4)], inv) for b in range(4)]
    out = [None] * 16
    for c in range(4):
        col = _dft4([_twiddle16(t[b][c], b * c, inv) for b in range(4)], inv)
        for d in range(4):
            out[c + 4 * d] = col[d]
    return out


def _dot(a, b):
    return jnp.dot(a, b, preferred_element_type=F32)


def _mean(v):
    return jnp.sum(v, axis=-1, keepdims=True) * (1.0 / D)


def _colsum8(v):
    return jnp.sum(v.reshape(v.shape[0] // 8, 8, v.shape[1]), axis=0)


def _wide(v):
    return jnp.concatenate([v] * (D // 128), axis=1)


def _layernorm_bwd(dxhat, xhat, rstd):
    return rstd * (dxhat - _mean(dxhat) - xhat * _mean(dxhat * xhat))


def _ds(start, size):
    return pl.ds(start if isinstance(start, int) else pl.multiple_of(start, size), size)


class _Packed:
    def __init__(self, ref):
        self.ref = ref

    @staticmethod
    def _index(idx, packing):
        lead, rows, cols = (idx + (slice(None),))[:3] if isinstance(idx, tuple) else (idx, slice(None), slice(None))
        if isinstance(rows, tuple):
            rows = _ds(rows[0] * (rows[1] // packing), rows[1] // packing)
        elif rows != slice(None):
            rows = slice(rows.start // packing, rows.stop // packing)
        return lead, rows, cols

    def __getitem__(self, idx):
        return pltpu.bitcast(self.ref[self._index(idx, 2)], BF16)

    def __setitem__(self, idx, value):
        lead, rows, cols = self._index(idx, 1)
        self.ref.at[lead].bitcast(BF16)[rows, cols] = value.astype(BF16)


def _loop(name, lo, hi, streams):
    def body(i, carry):
        _weave(*streams(i))
        return carry
    with jax.named_scope(name):
        jax.lax.fori_loop(lo, hi, body, 0)


def _once(name, *streams):
    with jax.named_scope(name):
        _weave(*streams)


def _weave(*streams):
    steps = sorted(((k + 0.5) / n, s) for s, (_, n) in enumerate(streams) for k in range(n))
    for _, s in steps:
        next(streams[s][0])
    for gen, _ in streams:
        assert next(gen, 1) == 1


def _dot_nt(a, b):
    return jax.lax.dot_general(a, b, (((1,), (1,)), ((), ())), preferred_element_type=F32)


def _dot_tn(a, b):
    return jax.lax.dot_general(a, b, (((0,), (0,)), ((), ())), preferred_element_type=F32)


def _unpack(u):
    return pltpu.bitcast(u << 16, F32), pltpu.bitcast(u & jnp.uint32(0xFFFF0000), F32)


def _pack(lo, hi):
    lo = pltpu.bitcast(lo.astype(BF16).astype(F32), U32) >> 16
    return lo | pltpu.bitcast(hi.astype(BF16).astype(F32), U32)


def _lhs(a11, a12, a21, a22):
    return [a11 + a22, a21 + a22, a11, a22, a11 + a12, a21 - a11, a12 - a22]


def _rhs(b11, b12, b21, b22):
    return [b11 + b22, b11, b12 - b22, b21 - b11, b22, b11 + b12, b21 + b22]


def _out(m):
    return m[0] + m[3] - m[4] + m[6], m[2] + m[4], m[1] + m[3], m[0] - m[1] + m[2] + m[5]


def _out_t(c11, c12, c21, c22):
    return [c11 + c22, c21 - c22, c12 + c22, c11 + c21, c12 - c11, c22, c11]


def _lhs_t(m):
    return m[0] + m[2] + m[4] - m[5], m[4] + m[6], m[1] + m[5], m[0] + m[1] + m[3] - m[6]


def _rhs_t(m):
    return m[0] + m[1] - m[3] + m[5], m[2] + m[5], m[3] + m[6], m[0] - m[2] + m[4] + m[6]


def _kernel(x_hbm, wr_hbm, wi_hbm, wg_hbm, wu_hbm, wd_hbm, c_ref, wm_hbm, g_hbm,
            ce_ref, co_ref, ft_ref,
            out_hbm, dx_hbm, dwr_hbm, dwi_hbm, dwg_hbm, dwu_hbm, dwd_hbm, dc_ref, dwm_hbm,
            x32, g32, w32, wn_v, wg_v, wu_v, wd_v, wm_v, ms_v,
            xp_v, gp_v, y_v, v_v, u_v, xs_v, y1_v, x2_v,
            wgu_s, wd_s, h_s, ht_s, dy_s, dyt_s, da_v, a_s, dgu_s,
            mod_v, acc_v, dwn_v, stat_v, t_v, sem):
    (ms_v, y_v, v_v, u_v, wgu_s, wd_s, h_s, ht_s, dy_s, dyt_s, da_v, a_s, dgu_s) = map(_Packed, (
        ms_v, y_v, v_v, u_v, wgu_s, wd_s, h_s, ht_s, dy_s, dyt_s, da_v, a_s, dgu_s))
    groups = []

    def copy(*pairs):
        group = [pltpu.make_async_copy(src, dst, sem.at[len(groups)]) for src, dst in pairs]
        groups.append(group)
        return group

    def start(*new):
        for group in new:
            for cp in group:
                cp.start()

    def wait(*started):
        for group in started:
            for cp in group:
                cp.wait()

    tile = lambda q: slice(128 * q, 128 * q + 128)
    col = lambda j, n=1: slice(D * j, D * (j + n))
    ld_wm = lambda j, n: copy((wm_hbm.at[:, col(j, n)], wm_v.at[:, col(j, n)]))
    ld_wm0, ld_wm2 = ld_wm(0, 2), ld_wm(2, 4)
    ld_x = [copy(*[(x_hbm.at[XC * k:XC * k + XC, tile(q)], x32.at[q, XC // 2 * k:XC // 2 * (k + 1)].bitcast(BF16))
                   for q in range(4)]) for k in range(S // XC)]
    ld_g = copy(*[(g_hbm.at[:, tile(q)], g32.at[q].bitcast(BF16)) for q in range(4)])
    ld_wd = copy((wd_hbm, wd_v))
    ld_w = copy(*[(w.at[0:256, tile(k)], w32.at[part, k].bitcast(BF16))
                  for part, w in enumerate((wr_hbm, wi_hbm)) for k in range(R)],
                (wr_hbm.at[256:DF], wn_v.at[0]), (wi_hbm.at[256:DF], wn_v.at[1]))
    ld_wgu = copy((wg_hbm, wg_v), (wu_hbm, wu_v))
    st_out = copy(*[(x32.at[q].bitcast(BF16), out_hbm.at[:, tile(q)]) for q in range(4)])
    st_dx = copy(*[(g32.at[q].bitcast(BF16), dx_hbm.at[:, tile(q)]) for q in range(4)])
    st_dw = copy(*[(w32.at[part, k].bitcast(BF16), w.at[0:256, tile(k)])
                   for part, w in enumerate((dwr_hbm, dwi_hbm)) for k in range(R)],
                 (dwn_v.at[0], dwr_hbm.at[256:DF]), (dwn_v.at[1], dwi_hbm.at[256:DF]))
    st_dwm = copy((wm_v, dwm_hbm))
    st_dwgu = copy((wg_v, dwg_hbm), (wu_v, dwu_hbm))
    dwgu_sem = sem.at[len(groups) - 1]
    st_dwd = copy((wd_v, dwd_hbm))

    first_row = lambda n=8: jax.lax.broadcasted_iota(jnp.int32, (n, 128), 0) == 0
    pair_rows = lambda p: pl.ds(p, N2, stride=R // 2)
    load_pairs = lambda ref, p: jnp.concatenate([ref[q, pair_rows(p), :] for q in range(4)], axis=1)

    def store_pairs(ref, p, u):
        for q in range(4):
            ref[q, pair_rows(p), :] = u[:, tile(q)]

    def silu():
        c = c_ref[...].astype(F32)
        sig = jax.nn.sigmoid(c)
        return (c * sig).astype(BF16), sig * (1.0 + c * (1.0 - sig))

    def modulate(j, n):
        mod_v[:, col(j, n)] = _dot(jnp.broadcast_to(silu()[0], (16, D)), wm_v[:, col(j, n)])[0:8]

    mod = lambda j: mod_v[0:1, col(j)]

    def accum(j, v):
        acc_v[:, j * D:(j + 1) * D] += _colsum8(v)

    def layernorm(layer, half, rows, x):
        mean = _mean(x)
        xc = x - mean
        rstd = jax.lax.rsqrt(_mean(xc * xc) + EPS)
        for k, v in enumerate((mean, rstd)):
            stat_v[2 * layer + k, half, rows, :] = jnp.broadcast_to(v, (x.shape[0], 128))
        return xc * rstd

    def layernorm_again(layer, half, rows, x):
        mean, rstd = (_wide(stat_v[2 * layer + k, half, rows, :]) for k in range(2))
        return (x - mean) * rstd, rstd

    def spectral_in(p, half, h):
        h0, h1, h2, h3 = (h[:, tile(q)] for q in range(4))
        s02, s13 = h0 + h2, h1 + h3
        yee = _dot_nt(ce_ref[0], (s02 + s13).astype(BF16))
        yeo = _dot_nt(ce_ref[1], (s02 - s13).astype(BF16))
        yo = _dot_nt(co_ref[...], jnp.concatenate([h0 - h2, h1 - h3], axis=1).astype(BF16))
        re = jnp.concatenate([yee[0:64], yeo[0:64], yo[0:128]], axis=0)
        im = jnp.concatenate([jnp.where(first_row(), 0.0, yee[64:72]), yee[72:128], yeo[64:128], yo[128:256]], axis=0)
        for k, v in enumerate((re, im, re + im)):
            y_v[p, 256 * k:256 * k + 256, tile(half)] = v
        y_v[p, 768:784, tile(half)] = jnp.where(first_row(16), yee[64:80], 0.0)

    def spectral_out(p, half):
        pee, peo = _dot_tn(u_v[p, 0:128, tile(half)], ce_ref[2]), _dot_tn(u_v[p, 128:256, tile(half)], ce_ref[1])
        po = _dot_tn(u_v[p, 256:D, tile(half)], co_ref[...])
        s, d = pee + peo, pee - peo
        return jnp.concatenate([s + po[:, 0:128], d + po[:, 128:256],
                                s - po[:, 0:128], d - po[:, 128:256]], axis=1)

    def filter_rows(t, w, slot, backward):
        z = _dft16([(v[:, 0:128], v[:, 128:256]) for v in t], False)
        y, dw = [], []
        for k1 in range(R):
            (zr, zi), (wr, wi) = z[k1], w(k1)
            if backward:
                xr, xi = xs_v[k1, slot, 0:128], xs_v[k1, slot, 128:256]
                dw.append((zr * xr + zi * xi, zi * xr - zr * xi))
                y.append((zr * wr + zi * wi, zi * wr - zr * wi))
            else:
                xs_v[k1, slot, 0:128] = zr
                xs_v[k1, slot, 128:256] = zi
                y.append((zr * wr - zi * wi, zr * wi + zi * wr))
        return _dft16(y, True), dw

    def tokens_fwd(p):
        for half in range(2):
            n1, last = 2 * p + half, y_v[p, 768:784, tile(half)]
            re, im, both = (jnp.concatenate([y_v[p, 256 * k:256 * k + 256, tile(half)], w], axis=0)
                            for k, w in enumerate((last, jnp.zeros_like(last), last)))
            k = _dot(both, ms_v[n1, :, 0:128])
            t_v[n1, :, 0:128] = (k - _dot(im, ms_v[n1, :, 128:256]))[0:264]
            t_v[n1, :, 128:256] = (k + _dot(re, ms_v[n1, :, 256:384]))[0:264]
            yield

    def tokens_inv(p):
        for half in range(2):
            n1 = 2 * p + half
            k = _dot_nt(v_v[n1, :, tile(2)], ms_v[n1, :, 0:128])
            u = (k + _dot_nt(v_v[n1, :, tile(1)], ms_v[n1, :, 256:384]),
                 k - _dot_nt(v_v[n1, :, tile(0)], ms_v[n1, :, 128:256]))
            even, odd = ([[v[16 * c + 8 * j:16 * c + 8 * j + 8] for c in range(16)] for v in u] for j in range(2))
            even[1][0] = jnp.where(first_row(), u[0][256:264], even[1][0])
            u_v[p, :, tile(half)] = jnp.concatenate(
                even[0][:8] + even[1][:8] + even[0][8:] + even[1][8:] + odd[0] + odd[1], axis=0)
            yield

    def keep(c, first, second):
        for n1 in range(R):
            vr, vi = (jnp.concatenate([first[n1][k], second[n1][k]], axis=0) for k in range(2))
            v_v[n1, (c, 16)] = jnp.concatenate([vr, vi, vr + vi], axis=1)

    def filter_words(c, backward):
        words = pl.ds(16 * (c % 8) + c // 8, 8, stride=2)
        ys, dws = [], []
        for odd in range(2):
            rows = _ds(128 * odd + 8 * c, 8)
            w = lambda k1: tuple(_unpack(w32[part, k1, words, :])[odd] for part in range(2))
            y, dw = filter_rows([t_v[n1, rows] for n1 in range(R)], w, rows, backward)
            t_v[0, rows, 0:128] = y[R - 1][0]
            ys.append(y)
            dws.append(dw)
        keep(c, *ys)
        if backward:
            weight = jnp.where(jax.lax.broadcasted_iota(jnp.int32, (8, 128), 0) + c == 0, 0.5, 1.0)
            for k1 in range(R):
                for part in range(2):
                    w32[part, k1, words, :] = _pack(weight * dws[0][k1][part], dws[1][k1][part])
        yield

    def filter_last(backward):
        w = lambda k1: tuple(jnp.broadcast_to(wn_v[part, :, tile(k1)].astype(F32), (8, 128)) for part in range(2))
        y, dw = filter_rows([t_v[n1, 256:264] for n1 in range(R)], w, slice(256, 264), backward)
        keep(16, y, [(jnp.zeros((8, 128), F32),) * 2] * R)
        if backward:
            for part in range(2):
                dwn_v[part] = (0.5 * jnp.concatenate([v[part][0:1] for v in dw], axis=1)).astype(BF16)
        yield

    def fwd_stats(i):
        for p in range(R // 2):
            u = jnp.concatenate([x32[q, pl.ds(N2 * i + p, 16, stride=R // 2), :] for q in range(4)], axis=1)
            xp_v[p, _ds(16 * i, 16), :] = u
            for half, xf in enumerate(_unpack(u)):
                layernorm(0, half, _ds(N2 * p + 16 * i, 16), xf)
        yield

    def fwd_in(p):
        for half, xf in enumerate(_unpack(xp_v[p])):
            xhat, _ = layernorm_again(0, half, _ds(N2 * p, N2), xf)
            spectral_in(p, half, xhat * (1.0 + mod(1)) + mod(0))
            yield

    def prep_wd(i):
        for k in range(8):
            quad = [wd_v[_ds(FH * a + 128 * i + 16 * k, 16), DH * b:DH * b + DH].astype(F32)
                    for a in range(2) for b in range(2)]
            for r, v in enumerate(_rhs(*quad)):
                wd_s[r, (8 * i + k, 16)] = v
        yield

    def prep_wgu(i):
        for k in range(2):
            for cols in (slice(lo, lo + 256) for lo in range(0, F, 256)):
                quad = [w[_ds(DH * a + 32 * i + 16 * k, 16), cols].astype(F32)
                        for a in range(2) for w in (wg_v, wu_v)]
                quad[1], quad[3] = 0.5 * quad[1], 0.5 * quad[3]
                for r, v in enumerate(_rhs(*quad)):
                    wgu_s[r, (2 * i + k, 16), cols] = v
        yield

    def prep_dy(p):
        rows = _ds(N2 * p, N2)
        u = load_pairs(g32, p)
        gp_v[p] = u
        top, bot = (v * mod(5) for v in _unpack(u))
        quad = (top[:, 0:DH], top[:, DH:D], bot[:, 0:DH], bot[:, DH:D])
        for r, v in enumerate(_out_t(*quad)):
            dy_s[r, (p, N2)] = v
        for r, v in enumerate(_out_t(*[t.T for t in quad])):
            dyt_s[r, :, rows] = v
        yield

    def ffn_da(p):
        for j in range(FH // 128):
            quad = _lhs_t([_dot_nt(dy_s[r, (p, N2)], wd_s[r, (j, 128)]) for r in range(7)])
            for k in range(4):
                da_v[k, (p, N2), tile(j)] = quad[k]
            yield

    def fwd_out(p):
        rows = _ds(N2 * p, N2)
        h = []
        for half, xf in enumerate(_unpack(xp_v[p])):
            y1 = spectral_out(p, half)
            yield
            y1_v[half, rows, :] = y1
            x2 = xf + (SCALE * mod(2)) * y1
            x2_v[half, rows, :] = x2
            xhat = layernorm(1, half, rows, x2)
            h.append(xhat * (1.0 + mod(4)) + mod(3))
        quad = (h[0][:, 0:DH], h[0][:, DH:D], h[1][:, 0:DH], h[1][:, DH:D])
        for r, v in enumerate(_lhs(*quad)):
            h_s[r, (p, N2)] = v
        for r, v in enumerate(_lhs(*[t.T for t in quad])):
            ht_s[r, :, rows] = v
        yield

    def geglu(g, uh, da):
        g2 = g * g
        m = _G1 * g2
        t = jnp.tanh(g * (_G0 + m))
        w = 1.0 + t
        gw = g * w
        z = w + (gw * (1.0 - t)) * (_G0 + 3.0 * m)
        return gw * uh, (da * uh) * z, da * gw

    def ffn_up(i, j):
        rows, cols = (i, TP), _ds(128 * j, 128)
        a = [None] * 4
        for fh in range(2):
            fcols = _ds(FH * fh + 128 * j, 128)
            m = [_dot(h_s[r, rows], wgu_s[r, :, fcols]) for r in range(7)]
            yield
            gt, ut, gb, ub = _out(m)
            a[fh], dgt, dut = geglu(gt, ut, da_v[fh, rows, cols].astype(F32))
            a[2 + fh], dgb, dub = geglu(gb, ub, da_v[2 + fh, rows, cols].astype(F32))
            for r, v in enumerate(_out_t(dgt, dut, dgb, dub)):
                dgu_s[r, rows, fcols] = v
        for r, v in enumerate(_lhs(*a)):
            a_s[r, rows, cols] = v
        yield

    def ffn_down(p):
        rows = _ds(N2 * p, N2)
        halves = lambda quad: [jnp.concatenate(quad[k:k + 2], axis=1) for k in (0, 2)]
        gout = _unpack(gp_v[p])
        dh = halves(_lhs_t([_dot_nt(dgu_s[r, (p, N2)], wgu_s[r]) for r in range(7)]))
        y2 = halves(_out([_dot(a_s[r, (p, N2)], wd_s[r]) for r in range(7)]))
        outs = []
        for half in range(2):
            x2 = x2_v[half, rows, :]
            xhat, rstd = layernorm_again(1, half, rows, x2)
            accum(3, dh[half])
            accum(4, dh[half] * xhat)
            dx2 = gout[half] + _layernorm_bwd(dh[half] * (1.0 + mod(4)), xhat, rstd)
            accum(2, dx2 * y1_v[half, rows, :])
            x2_v[half, rows, :] = dx2
            spectral_in(p, half, dx2 * (SCALE * mod(2)))
            outs.append(x2 + mod(5) * y2[half])
        for half in range(2):
            accum(5, gout[half] * y2[half])
        store_pairs(x32, p, _pack(*outs))

    def bwd_out(p):
        dx = []
        for half, xf in enumerate(_unpack(xp_v[p])):
            dh1 = spectral_out(p, half)
            yield
            xhat, rstd = layernorm_again(0, half, _ds(N2 * p, N2), xf)
            accum(0, dh1)
            accum(1, dh1 * xhat)
            dx.append(x2_v[half, _ds(N2 * p, N2), :] + _layernorm_bwd(dh1 * (1.0 + mod(1)), xhat, rstd))
        store_pairs(g32, p, _pack(*dx))
        yield

    def mod_grads(j, n):
        dmod = jnp.sum(acc_v[:, col(j, n)], axis=0, keepdims=True)
        mod_v[:, col(j)] = _dot_nt(jnp.broadcast_to(dmod.astype(BF16), (16, n * D)), wm_v[:, col(j, n)])[0:8]
        silu_col = jnp.broadcast_to(silu()[0].astype(F32), (128, D)).T
        for k in range(n * D // 128):
            wm_v[:, tile(j * D // 128 + k)] = (silu_col * dmod[:, tile(k)]).astype(BF16)
        yield

    def dw_down(j):
        m = []
        for r in range(7):
            m.append(_dot(dyt_s[r], a_s[r, :, _ds(128 * j, 128)]))
            yield
        for k, v in enumerate(_rhs_t(m)):
            wd_v[_ds(FH * (k // 2) + 128 * j, 128), DH * (k % 2):DH * (k % 2) + DH] = v.T.astype(BF16)
        yield

    def dw_gate_up(j):
        m = []
        for r in range(7):
            m.append(_dot(ht_s[r], dgu_s[r, :, _ds(128 * j, 128)]))
            yield
        for k, (w, v) in enumerate(zip((wg_v, wu_v, wg_v, wu_v), _rhs_t(m))):
            w[DH * (k // 2):DH * (k // 2) + DH, _ds(128 * j, 128)] = (0.5 * v if k % 2 else v).astype(BF16)
        for w, dst in ((wg_v, dwg_hbm), (wu_v, dwu_hbm)):
            cols = _ds(128 * j, 128)
            pltpu.make_async_copy(w.at[:, cols], dst.at[:, cols], dwgu_sem).start()
        yield

    def prep_dft(n1):
        fr, fi = ft_ref[0:N2, 0:128], ft_ref[0:N2, 128:256]
        tr, ti = (ft_ref[_ds(N2 + 8 * n1, 8), tile(part)][0:1] for part in range(2))
        mr, mi = fr * tr - fi * ti, fr * ti + fi * tr
        ms_v[n1] = jnp.concatenate([mr, mr + mi, mi - mr], axis=1)
        yield

    def chain(stage, chunks, first, count):
        return (None for k in range(count) for _ in stage(first + k)), chunks * count

    with jax.named_scope("init"):
        start(*ld_x, ld_wm0, ld_wd, ld_w, ld_wm2, ld_g, ld_wgu)
        acc_v[...] = jnp.zeros(acc_v.shape, F32)
        jax.lax.fori_loop(0, R, lambda n1, carry: next(prep_dft(n1), None), None)

    def stats(i):
        for k, group in enumerate(ld_x):
            pl.when(i == k * (XC // 2 // N2))(lambda: wait(group))
        return [(fwd_stats(i), 1)]
    _loop("stats", 0, P // N2, stats)
    wait(ld_wm0)
    modulate(0, 2)
    _loop("in0", 0, R // 4, lambda i: [chain(fwd_in, 2, 2 * i, 2)])
    wait(ld_wd)
    _loop("s_fwd", 0, R // 2, lambda p: [(tokens_fwd(p), 2), (prep_wd(jnp.minimum(p, FH // 128 - 1)), 1)])
    wait(ld_w)
    _loop("filter", 0, 16, lambda c: [(filter_words(c, False), 1)])
    _once("filter", (filter_last(False), 1))
    wait(ld_wm2, ld_g)
    modulate(2, 4)
    _loop("s_inv", 0, R // 2, lambda p: [(tokens_inv(p), 2), (prep_dy(p), 1)])
    wait(ld_wgu)
    _loop("out", 0, R // 2, lambda p: [(ffn_da(p), 7), (fwd_out(p), 3), (prep_wgu(p), 1)])

    def ffn(i, carry):
        _weave(chain(lambda j: ffn_up(i, j), 3, 0, FH // 128))
        for p in (2 * i, 2 * i + 1):
            ffn_down(p)
        for p in (2 * i, 2 * i + 1):
            _weave((tokens_fwd(p), 2))
        return carry
    jax.lax.fori_loop(0, P // TP, ffn, 0)
    start(st_out)
    _loop("bfilter", 0, 16, lambda c: [(filter_words(c, True), 1)])
    _once("bfilter", (filter_last(True), 1))
    start(st_dw)
    _once("s_inv2", chain(tokens_inv, 2, 0, 2))
    _loop("bout", 0, 3, lambda i: [chain(dw_down, 8, i, 1), chain(bwd_out, 3, 2 * i, 2),
                                   chain(tokens_inv, 2, 2 * i + 2, 2)])
    _once("bout", chain(dw_down, 8, 3, 1), chain(bwd_out, 3, 6, 2), (mod_grads(3, 3), 1))
    start(st_dx)
    acc_v[:, col(2)] = SCALE * acc_v[:, col(2)]
    _once("dmod", chain(dw_down, 8, 4, 1), (mod_grads(0, 3), 1))
    dsilu = mod_v[0:1, col(0)] + mod_v[0:1, col(3)]
    dc_ref[...] = (dsilu * silu()[1]).astype(BF16)
    start(st_dwm)
    _loop("dwd", 5, FH // 128, lambda j: [(dw_down(j), 8)])
    start(st_dwd)
    _loop("dwgu", 0, F // 256, lambda j: [chain(dw_gate_up, 8, 2 * j, 2)])
    with jax.named_scope("drain"):
        wait(st_out, st_dw, st_dx, st_dwm, st_dwd, st_dwgu)


@jax.jit
def pallas_adaLN_cond__spectral_gfnet__geglu_ffn__prompt_kernel(
    A_x: jax.Array,
    A_w_r: jax.Array,
    A_w_i: jax.Array,
    B_x: jax.Array,
    B_w_gate: jax.Array,
    B_w_up: jax.Array,
    B_w_down: jax.Array,
    c: jax.Array,
    w_mod: jax.Array,
    grad_out: jax.Array,
):
    del B_x
    hbm = pl.BlockSpec(memory_space=pltpu.HBM)
    vmem = pl.BlockSpec(memory_space=pltpu.VMEM)
    sds = lambda *s: jax.ShapeDtypeStruct(s, BF16)
    v = pltpu.VMEM
    pk = lambda n, rows, cols: v((n, rows // 2, cols), U32)
    outs = pl.pallas_call(
        _kernel,
        in_specs=[hbm] * 6 + [vmem] + [hbm] * 2 + [vmem] * 3,
        out_specs=[hbm] * 7 + [vmem, hbm],
        out_shape=[sds(S, D), sds(S, D), sds(DF, S), sds(DF, S), sds(D, F), sds(D, F), sds(F, D),
                   sds(1, D), sds(D, 6 * D)],
        scratch_shapes=[
            v((4, P, 128), U32), v((4, P, 128), U32),
            v((2, R, 128, 128), U32), v((2, 1, S), BF16),
            v((D, F), BF16), v((D, F), BF16), v((F, D), BF16), v((D, 6 * D), BF16),
            pk(R, N2, 384),
            v((R // 2, N2, D), U32), v((R // 2, N2, D), U32),
            pk(R // 2, 784, 256), pk(R, 272, 384), pk(R // 2, D, 256), v((R, 264, 256), F32),
            v((2, P, D), F32), v((2, P, D), F32),
            pk(7, DH, F), pk(7, FH, DH),
            pk(7, P, DH), pk(7, DH, P),
            pk(7, P, DH), pk(7, DH, P),
            pk(4, P, FH), pk(7, P, FH), pk(7, P, F),
            v((8, 6 * D), F32), v((8, 6 * D), F32),
            v((2, 1, S), BF16),
            v((4, 2, P, 128), F32), v((R, 264, 256), F32),
            pltpu.SemaphoreType.DMA((24,)),
        ],
        compiler_params=pltpu.CompilerParams(vmem_limit_bytes=127 * 1024 * 1024),
    )(A_x.reshape(S, D), A_w_r.T, A_w_i.T, B_w_gate, B_w_up, B_w_down, c, w_mod,
      grad_out.reshape(S, D), _CE, _CO, _FT)
    return (outs[0].reshape(1, S, D), outs[1].reshape(1, S, D), outs[2].T, outs[3].T, *outs[4:])
```
